```python
import os as _os
_os.environ.setdefault('JAX_PLATFORMS', 'cpu')
import jax
import jax.numpy as jnp

def _softmax(x, axis=-1):
    return jax.nn.softmax(x, axis=axis)

def _gelu(x):
    return jax.nn.gelu(x, approximate=True)

def _silu(x):
    return jax.nn.silu(x)

def _sigmoid(x):
    return jax.nn.sigmoid(x)

def _layernorm(x, axis=-1, eps=1e-05):
    m = jnp.mean(x, axis=axis, keepdims=True)
    v = jnp.var(x, axis=axis, keepdims=True)
    return (x - m) / jnp.sqrt(v + eps)

def _scatter_add(tgt, idx, src, axis=0):
    return tgt.at[idx].add(src)

def _segment_sum(src, seg, n):
    return jax.ops.segment_sum(src, seg, n)

class _Rng:

    def __init__(self, key):
        self._k = key

    def _next(self):
        self._k, sub = jax.random.split(self._k)
        return sub

    def normal(self, shape):
        return jax.random.normal(self._next(), shape, dtype=jnp.bfloat16)

    def randint(self, lo, hi, shape):
        return jax.random.randint(self._next(), shape, lo, hi, dtype=jnp.int32)

    def uniform(self, shape, lo=0.0, hi=1.0):
        return jax.random.uniform(self._next(), shape, jnp.bfloat16, lo, hi)

    def permutation(self, n):
        return jax.random.permutation(self._next(), n)
kernel_name = 'adaLN_cond__sliding_local_dilated__dense_activation_gelu__prompt'

def setup_inputs():
    _rng = _Rng(jax.random.key(int.from_bytes(__import__("os").urandom(4), "little")))
    _w = lambda a: (lambda t: t.astype(jnp.bfloat16) if jnp.issubdtype(t.dtype, jnp.floating) else t)(jnp.asarray(a))

    def _A_setup():
        B, S, D = (1, 2048, 576)
        return {'x': _w((lambda *s: _rng.normal(s) * 0.05)(B, S, D)), 'wqkv': _w((lambda *s: _rng.normal(s) * 0.05)(D, 3 * D)), 'wo': _w((lambda *s: _rng.normal(s) * 0.05)(D, D))}
    _A_in = _A_setup()

    def _B_setup():
        B, S, D, F = (1, 2048, 576, 4608)
        return {'x': _w((lambda *s: _rng.normal(s) * 0.05)(B, S, D)), 'w1': _w((lambda *s: _rng.normal(s) * 0.8)(D, F) * D ** (-0.5)), 'b1': _w((lambda *s: _rng.normal(s) * 0.8)(F) * 0.01), 'w2': _w((lambda *s: _rng.normal(s) * 0.8)(F, D) * F ** (-0.5)), 'b2': _w((lambda *s: _rng.normal(s) * 0.8)(D) * 0.01)}
    _B_in = _B_setup()
    return {'A_x': _A_in['x'], 'A_wqkv': _A_in['wqkv'], 'A_wo': _A_in['wo'], 'B_x': _B_in['x'], 'B_w1': _B_in['w1'], 'B_b1': _B_in['b1'], 'B_w2': _B_in['w2'], 'B_b2': _B_in['b2'], 'c': _w((lambda *s: _rng.normal(s) * 0.05)(1, 576) * 8.0), 'w_mod': _w((lambda *s: _rng.normal(s) * 0.05)(576, 6 * 576) * 576 ** (-0.5) * 8.0)}

def reference(A_x, A_wqkv, A_wo, B_x, B_w1, B_b1, B_w2, B_b2, c, w_mod):

    def _A_ref(x, wqkv, wo):
        B, S, D = x.shape
        H = 32
        Dh = D // H
        W, dil = (8, 2)
        qkv = (lambda x, *d: x.transpose(*d))((x @ wqkv).reshape(B, S, 3, H, Dh), 2, 0, 3, 1, 4)
        q, k, v = (qkv[0], qkv[1], qkv[2])
        scale = Dh ** (-0.5)
        pos = jnp.arange(S)
        off = jnp.arange(W) * dil
        idx = pos[:, None] - off[None, :]
        mask = idx >= 0
        idx_c = jnp.where(mask, idx, 0).reshape(-1)
        kg = k[:, :, idx_c, :].reshape(B, H, S, W, Dh)
        vg = v[:, :, idx_c, :].reshape(B, H, S, W, Dh)
        logits = jnp.einsum('bhsd,bhswd->bhsw', q, kg) * scale
        logits = jnp.where(mask[None, None, :, :], logits, -1000000000.0)
        attn = _softmax(logits, axis=-1)
        o = jnp.einsum('bhsw,bhswd->bhsd', attn, vg)
        return (lambda x, *d: x.transpose(*d))(o, 0, 2, 1, 3).reshape(B, S, D) @ wo

    def _B_ref(x, w1, b1, w2, b2):
        h = jnp.einsum('bsd,df->bsf', x, w1) + b1
        h = _gelu(h)
        return jnp.einsum('bsf,fd->bsd', h, w2) + b2
    x = A_x
    mod = (_silu(c) @ w_mod).reshape(c.shape[0], 6, 1, -1)
    sa, ca, ga, sb, cb, gb = (mod[:, 0].copy(), mod[:, 1].copy(), mod[:, 2].copy(), mod[:, 3].copy(), mod[:, 4].copy(), mod[:, 5].copy())
    h = _layernorm(x, axis=-1) * (1 + ca) + sa
    x = x + ga * _A_ref(h, A_wqkv, A_wo)
    h = _layernorm(x, axis=-1) * (1 + cb) + sb
    x = x + gb * _B_ref(h, B_w1, B_b1, B_w2, B_b2)
    return x
```

```python
import collections
import contextlib
import functools
import jax
import jax.numpy as jnp
from jax import lax
import jax.experimental.pallas as pl
import jax.experimental.pallas.tpu as pltpu

S, D, F = 2048, 576, 4608
H, DH, W, DIL = 32, 18, 8, 2
DP = 640
TM = 512
NB = S // TM
NC = F // 512
EPS = 1e-5
C0 = 0.7978845608028654
C1 = C0 * 0.044715
f32, bf16, u32 = jnp.float32, jnp.bfloat16, jnp.uint32
NT = (((1,), (1,)), ((), ()))


def tmap(f, *xs):
    if isinstance(xs[0], (list, tuple)):
        return [tmap(f, *ys) for ys in zip(*xs)]
    return f(*xs)


add = lambda a, b: tmap(lambda x, y: x + y, a, b)
sub = lambda a, b: tmap(lambda x, y: x - y, a, b)


def enc_a1(kind, a11, a12, a21, a22):
    if kind == "W":
        s1 = add(a21, a22); s2 = sub(s1, a11); s3 = sub(a11, a21); s4 = sub(a12, s2)
        return [a11, a12, s4, a22, s1, s2, s3]
    return [add(a11, a22), add(a21, a22), a11, a22, add(a11, a12), sub(a21, a11), sub(a12, a22)]


def enc_b1(kind, b11, b12, b21, b22):
    if kind == "W":
        t1 = sub(b12, b11); t2 = sub(b22, t1); t3 = sub(b22, b12); t4 = sub(t2, b21)
        return [b11, b21, b22, t4, t1, t2, t3]
    return [add(b11, b22), b11, sub(b12, b22), sub(b21, b11), b22, add(b11, b12), add(b21, b22)]


def encode(enc1, kinds, blk):
    L = len(kinds)
    if L == 0:
        yield blk(0, 0)
    elif L == 1:
        yield from enc1(kinds[0], blk(0, 0), blk(0, 1), blk(1, 0), blk(1, 1))
    else:
        quad = lambda R, C: [blk(2 * R + r, 2 * C + c) for r in range(2) for c in range(2)]
        for lv in enc1(kinds[0], quad(0, 0), quad(0, 1), quad(1, 0), quad(1, 1)):
            yield from enc1(kinds[1], *lv)


def dec1(kind, get, stash):
    if kind == "W":
        m0, u2, u3, u4 = {}, {}, {}, {}
        for k, v in get(0): m0[k] = stash(v, 0)
        for k, v in get(1): yield (0, k), m0[k]() + v
        for k, v in get(5): u2[k] = stash(m0[k]() + v, 1)
        for k, v in get(6): u3[k] = stash(u2[k]() + v, 0)
        for k, v in get(3): yield (2, k), u3[k]() - v
        for k, v in get(4):
            u4[k] = stash(u2[k]() + v, 0)
            yield (3, k), u3[k]() + v
        for k, v in get(2): yield (1, k), u4[k]() + v
    else:
        m0, m1, m2, a11, a22 = {}, {}, {}, {}, {}
        for k, v in get(0): m0[k] = stash(v, 0)
        for k, v in get(1):
            m1[k] = stash(v, 0); a22[k] = stash(m0[k]() - v, 1)
        for k, v in get(3):
            a11[k] = stash(m0[k]() + v, 0)
            yield (2, k), m1[k]() + v
        for k, v in get(6): a11[k] = stash(a11[k]() + v, 1)
        for k, v in get(2):
            m2[k] = stash(v, 0); a22[k] = stash(a22[k]() + v, 0)
        for k, v in get(4):
            yield (1, k), m2[k]() + v
            yield (0, k), a11[k]() - v
        for k, v in get(5): yield (3, k), a22[k]() + v


def decode(kinds, prod, stash):
    L = len(kinds)
    keep = lambda v, far: stash(v) if far else (lambda: v)
    if L == 0:
        yield (0, 0), prod(0)
    elif L == 1:
        for (q, _), v in dec1(kinds[0], lambda r: [(0, prod(r))], keep):
            yield (q // 2, q % 2), v
    else:
        inner = lambda a: dec1(kinds[1], lambda b: [(0, prod(7 * a + b))], keep)
        for (Q, (q, _)), v in dec1(kinds[0], inner, lambda v, far: stash(v)):
            yield (2 * (Q // 2) + q // 2, 2 * (Q % 2) + q % 2), v


class Sym:
    __add__ = __sub__ = lambda s, o: Sym()

    def __init__(self, rc=None):
        self.rc = rc


def slots(enc1, kinds):
    out, n = [], 0
    for e in encode(enc1, kinds, lambda r, c: Sym((r, c))):
        if e.rc is None:
            out.append(("enc", n)); n += 1
        else:
            out.append(("raw",) + e.rc)
    return out, (n + 1) // 2


PROG = """
> s0 x0 wm0 wm1 wm2 wq0
init
s0 x0 > wq1
st1.0
wm0 wm1 wm2 > wq2 s1 s2
mm.0 mod.0 ap1.0
wq0 > x1
pq.0
wq1 >
stream x2 x3 wo0 wm3 wm4 wm5 wm6 wm7 wm8 w10 w11 w12 w13 w14 w15 w16 w17 w18 w20 w21 w22 w23 w24 w25 w26 w27 w28
~2300 pq.1
qkv.0.0
wq2 x1 >
~2600 pq.2 st1.1
qkv.0.1
x2 >
~1500 ap1.1
~6800@1500 ln1.2 qk.0-2
qkv.0.2 !1 qkv.1.0-1
s1 s2 x3 wo0 wm3 wm4 wm5 wm6 wm7 wm8 >
~6700 pv.0-1 qk.3-4 pv.2-3 eo.0
~1800@6700 pwo mod.1
mm.1-2 qkv.1.2 qkv.2.0-1 !
~2600 mod.2 st1.3
proj.0
w10 w11 w12 w13 w14 w15 w16 w17 w18 >
~1300 ap1.3
~9900@1300 ln2.0 pw1.0-6
qkv.2.2 !1 qkv.3.0-2
w20 w21 w22 w23 w24 w25 w26 w27 w28 >
~2000 pw1.7-8
~16000@2000 gate pw2.0-4
f1.0.0-8 ! bar
~3700@1900 pw2.5-8
e2.0.32.5 !! bar
~6600 qk.5-8 pv.4-7 eo.1
f2.0.39 ! proj.1
~3000 ln2.1
f2.0.49 ! out.0.0
f1.1.0-8 bar e2.1.8.8 !! bar
~8800 qk.9-12 pv.8-11 eo.2
f2.1.35 ! proj.2
~4200 ln2.2
f2.1.49 ! out.1.0
f1.2.0-8 bar e2.2.8.8 !! bar
~8500 qk.13-15 pv.12-15 eo.3
f2.2.34 ! proj.3
~4500 ln2.3
f2.2.49 ! out.2.0
f1.3.0-8 bar e2.3.8.8 !! bar
f2.3.42 out.3.1-2 f2.3.49 out.3.3
"""


def build(K1="WW", K2="WW", KQ="", KO="", ST=1, SC=False, order=None, NS=40, flags=None, AD=1, PT=2060, LR=16, DEFER=7, AC=24, DA=24, NZ=3, HALF=1, PB=14, DR=2.36, NOB=False, TS=1.0, ONE=1, GR=1, PRI=0, DL=0, NOCSE=1, TIE=False):
    scope = (lambda n: jax.named_scope(n)) if SC else (lambda n: contextlib.nullcontext())
    nt = lambda k: 7 ** len(k) * (4 >> len(k))
    wshape = lambda k: (pltpu.VMEM((nt(k), (D >> len(k)) + 16, 128), bf16), pltpu.VMEM((1, D, 128), bf16))
    ashape = lambda k: (pltpu.VMEM((nt(k), (512 >> len(k)) + 16, 128), bf16), pltpu.VMEM((4, 128, 128), bf16))

    def kernel(c_hbm, b1_hbm, b2_hbm, x_hbm, wqkv_hbm, wo_hbm, w1_hbm, w2_hbm, wm_hbm, o_hbm,
               c_ref, b1_ref, b2_ref, xs, wqkv_s, wo_s, w1_s, w2_s, wm_s, out_s, tq, wo_f, wo_g, mr_s, modc, q_s, k_s, v_s, o_s, pp_s, far_s, p_s,
               x1_s, h2_s, he_s, hr_s, w1e, w1r, w2e, g0, g1, z_s, st_s, wa_s, ha_s, oa_s, sems, osem, zsem, bsem):
        nsem = [0]

        def cp(src, dst, c0, n):
            i = nsem[0]; nsem[0] += 1
            if n is None:
                return pltpu.make_async_copy(src, dst.at[pl.ds(0, D)], sems.at[i])
            return pltpu.make_async_copy(src.at[:, pl.ds(c0, n)], dst.at[pl.ds(0, D), pl.ds(c0, n)], sems.at[i])
        QC = (0, 640, 1152, 3 * D)
        small = [pltpu.make_async_copy(a, b, sems.at[35 + n]) for n, (a, b) in enumerate(((c_hbm, c_ref), (b1_hbm, b1_ref), (b2_hbm, b2_ref)))]
        cps = dict(s=small, wq=[cp(wqkv_hbm, wqkv_s, QC[t], QC[t + 1] - QC[t]) for t in range(3)], wm=[cp(wm_hbm, wm_s, t * 384, 384) for t in range(9)],
                   x=[cp(x_hbm, xs, i * TM, TM) for i in range(NB)], wo=[cp(wo_hbm, wo_s, 0, None)],
                   w1=[cp(w1_hbm, w1_s, j * 512, 512) for j in range(NC)],
                   w2=[cp(w2_hbm, w2_s, j * 512, 512) for j in range(NC)])

        def dma(waits, starts):
            with scope("dma_" + waits.replace(" ", "_")):
                for n in waits.split():
                    cps[n[:-1]][int(n[-1])].wait()
            for n in starts.split():
                cps[n[:-1]][int(n[-1])].start(priority=PRI)

        zero = pl.semaphore_read(zsem)
        clock = [0.0, 0]
        jobs = []
        last = {}

        due_list = collections.deque()

        def spare(ref):
            return (0,) * (len(ref.shape) - 2) + (pl.ds(pl.multiple_of(ref.shape[-2] - 16 + zero * 16, 16), 8), slice(0, 128))

        def release(ref, tok):
            if tok is not None:
                ref[spare(ref)] = pltpu.bitcast(tok, u32) if ref.dtype == u32 else tok.astype(ref.dtype)

        def written(ref):
            v = ref[spare(ref)]
            return pltpu.bitcast(v, f32) if ref.dtype == u32 else v.astype(f32)

        def tied(a):
            while due_list:
                a = jnp.concatenate([a[0:8] | (pltpu.bitcast(due_list.popleft(), u32) & zero.astype(u32)), a[8:]], axis=0)
            return pltpu.bitcast(a, bf16)

        def spawn(pieces, dur, delay=0):
            tot = sum(p[0] for p in pieces); t = clock[0] + delay; q = collections.deque()
            for p in pieces:
                q.append((t, p)); t += dur * p[0] / tot
            jobs.append(q)
            return q

        def run(p, tok):
            for r in (p[1] if isinstance(p[1], list) else [p[1]]):
                release(r, tok)
            return p[2]()

        def join(q, tie=False):
            while q:
                last[id(q)] = run(q.popleft()[1], None)
            res = last.pop(id(q), None)
            if tie and res is not None:
                due_list.append(res if isinstance(res, jax.Array) else written(res))

        def mm(a, b, dims=None):
            y = (jnp.dot(a, b, preferred_element_type=f32) if dims is None
                 else lax.dot_general(a, b, dims, preferred_element_type=f32))
            m, n = y.shape
            passes = (a.shape[1] // 128) * (n // 128)
            t0 = clock[0]; dt = m * passes / 4
            clock[0] += dt
            while True:
                due = [q for q in jobs if q and q[0][0] < (clock[0] if not ONE else t0 + m if clock[1] % 4 == 0 else -1)]
                if not due:
                    break
                q = min(due, key=lambda q: q[0][0])
                t, p = q.popleft()
                f = max(t - t0, 0.0) / dt
                if ONE:
                    f = max(t - t0, 0.0) / m
                elif passes < 4:
                    f = (clock[1] % 4 + f * passes) % 4 / 4
                r = min(int(f * m) // 8 * 8, m - 8)
                res = run(p, y[r:r + 8, 0:128])
                last[id(q)] = res
            clock[1] += passes
            return y

        def init():
            for r in jax.tree.leaves([st_s, pp_s, far_s, he_s, hr_s, g0, g1, w1e, w1r, w2e, wa_s, ha_s, oa_s]):
                r[(zero,) + (0,) * (len(r.shape) - 3) + (slice(0, 8), slice(0, 128))] = jnp.zeros((8, 128), r.dtype)
        if order:
            init()
        slot = [0, 0]

        def stash(v, pool=0):
            if not ST or v.shape[0] > 144 or v.shape[1] != 128:
                return lambda: v
            k = pool * NS + slot[pool] % NS; slot[pool] += 1
            st_s[k, 0:v.shape[0]] = v
            return lambda: st_s[k, 0:v.shape[0]]

        def col_of_row(row):
            return jnp.broadcast_to(row, (128, row.shape[1])).T

        def pad0(v, n, axis):
            sh = list(v.shape); sh[axis] = n - sh[axis]
            return jnp.concatenate([v, jnp.zeros(sh, v.dtype)], axis=axis)

        fold = lambda v: functools.reduce(jnp.add, [v[r:r + 8] for r in range(0, v.shape[0], 8)])
        P = functools.partial

        mcol = lambda i, r0, n: modc[i * D + r0:i * D + r0 + n, :]
        mrow = {}

        def mod_mm(part):
            cv = c_ref[...].astype(f32)
            act = jnp.broadcast_to(cv * jax.nn.sigmoid(cv), (16, D)).astype(bf16)
            y = jnp.dot(act, wm_s[0:D, part * 2 * D:(part + 1) * 2 * D], preferred_element_type=f32)[0:8]
            ch = lax.broadcasted_iota(jnp.int32, y.shape, 1) + part * 2 * D
            scale = ((ch >= D) & (ch < 2 * D)) | ((ch >= 4 * D) & (ch < 5 * D))
            mr_s[8 * part:8 * part + 8] = jnp.where(scale, y + 1.0, y)

        def mod_cols(part):
            def f(t):
                row = mr_s[8 * part:8 * part + 8, t * 128:(t + 1) * 128]
                modc[(9 * part + t) * 128:(9 * part + t + 1) * 128, :] = jnp.concatenate([row] * 16, axis=0).T
            return [(60, mr_s, P(f, t)) for t in range(9)]

        def ld(ref, ix, r0, n):
            return pltpu.bitcast(ref.bitcast(u32)[ix + (slice(r0 // 2, (r0 + n) // 2),)], bf16)

        def enc_w(kinds, load, dst, src):
            n = 2 ** len(kinds); rb = D // n; ct = 4 // n

            def f(r0):
                for k in range(ct):
                    for i, e in enumerate(encode(enc_a1, kinds, lambda r, c: load(r * rb + r0, 16, c * ct + k))):
                        dst[0][i * ct + k, r0:r0 + 16] = e.astype(bf16)
                for r in range(n):
                    dst[1][0, r * rb + r0:r * rb + r0 + 16] = load(r * rb + r0, 16, 4).astype(bf16)
                return dst[0]
            return [(15 * n * n, src, P(f, r0)) for r0 in range(0, rb, 16)]

        def enc_act(kinds, load, dst, src, cost):
            n = 2 ** len(kinds); rb = 512 // n; ct = 4 // n

            def f(r0):
                rows = [load(r * rb + r0, 16) for r in range(n)]
                for k in range(ct):
                    for i, e in enumerate(encode(enc_b1, kinds, lambda r, c: rows[r][c * ct + k])):
                        dst[0][i * ct + k, r0:r0 + 16] = e.astype(bf16)
                return dst[0]

            def tail(r0):
                for t, v in enumerate(load(512 + r0, 16)):
                    dst[1][t, r0:r0 + 16] = v.astype(bf16)
                    dst[1][t, 64 + r0:80 + r0] = jnp.zeros((16, 128), bf16)
            return ([(cost * n * 8, src, P(f, r0)) for r0 in range(0, rb, 16)]
                    + [(cost * 8, src, P(tail, r0)) for r0 in range(0, 64, 16)])

        def mm576(kinds, a, b):
            n = 2 ** len(kinds); rb = D // n; ct = 4 // n
            for t in range(ct):
                for m0 in range(0, rb, 144):
                    prod = lambda i: functools.reduce(jnp.add, [
                        mm(ld(a[0], (i * ct + k,), m0, 144), ld(b[0], (i * ct + t,), k * 128, 128)) for k in range(ct)])
                    for (r, c), v in decode(kinds, prod, stash):
                        yield r * rb + m0, (c * ct + t) * 128, v + mm(ld(a[1], (0,), r * rb + m0, 144), ld(b[1], (c * ct + t,), 0, 128))

        def prep_wqkv(part):
            c0, c1 = ((0, 640), (640, 1152), (1152, 3 * D))[part]

            def tr(kt):
                blk = wqkv_s[kt * 128:min(D, (kt + 1) * 128), c0:c1]
                tq[kt, c0 // 2:c1 // 2] = pltpu.bitcast((blk if kt < 4 else pad0(blk, 128, 0)).T, u32)

            def load(r0, n, kt):
                d, h0 = divmod(r0, H)
                u = tq[kt, pl.ds(part * (D // 2) + h0 * (DH // 2) + d // 2, n, stride=DH // 2), :]
                return pltpu.bitcast(u & u32(0xFFFF0000) if d % 2 else u << 16, f32)
            return [(100, wqkv_s, P(tr, kt)) for kt in range(5)] + enc_w(KQ, load, wa_s[part], tq)

        def prep_wo():
            def cvt(nt, r0):
                blk = wo_s[r0:r0 + 144, nt * 128:min(D, (nt + 1) * 128)].astype(f32)
                wo_f[nt, r0:r0 + 144] = blk if nt < 4 else pad0(blk, 128, 1)

            def tr(nt, kt):
                rows = [wo_f[nt, pl.ds(d, H, stride=DH), :] for d in range(4 * kt, min(DH, 4 * kt + 4))]
                wp = jnp.concatenate(rows, axis=0)
                n = min(128, D - nt * 128)
                wo_g[kt, nt * 128:nt * 128 + n] = (wp if kt < 4 else pad0(wp, 128, 0)).T[:n]
            return ([(40, wo_s, P(cvt, nt, r0)) for nt in range(5) for r0 in range(0, D, 144)] + [(60, wo_f, P(tr, nt, kt)) for nt in range(5) for kt in range(5)]
                    + enc_w(KO, lambda r0, n, kt: wo_g[kt, r0:r0 + n], wa_s[3], wo_g))

        def norm(load, src, shift_i, scale_i):
            st = {}

            def s1(r0):
                y = [fold(t) for t in load(r0, LR)]
                st["a"] = y if r0 == 0 else add(st["a"], y)
                if r0 == D - LR:
                    st["m"] = [jnp.sum(a, axis=0, keepdims=True) * (1.0 / D) for a in st["a"]]
                return st["a"][-1]

            def s2(r0):
                y = [fold((t - m) * (t - m)) for t, m in zip(load(r0, LR), st["m"])]
                st["a"] = y if r0 == 0 else add(st["a"], y)
                if r0 == D - LR:
                    st["r"] = [lax.rsqrt(jnp.sum(a, axis=0, keepdims=True) * (1.0 / D) + EPS) for a in st["a"]]
                return st["a"][-1]

            def out(r0, n):
                sc, sh = mcol(scale_i, r0, n), mcol(shift_i, r0, n)
                return [((t - m) * r) * sc + sh for t, m, r in zip(load(r0, n), st["m"], st["r"])]
            return ([(LR, src, P(s1, r0)) for r0 in range(0, D, LR)]
                    + [(2 * LR, src, P(s2, r0)) for r0 in range(0, D, LR)]), out

        def tiles(ref, c0):
            def load(r0, n):
                v = ref[r0:r0 + n, c0:c0 + TM].astype(f32)
                return [v[:, t * 128:(t + 1) * 128] for t in range(4)]
            return load

        n1 = {}

        def st1(i):
            ps, n1[i] = norm(tiles(xs, i * TM), xs, 0, 1)
            return ps

        ap1 = lambda i: enc_act(KQ, n1[i], ha_s[i % 3], xs, 6)
        ln1 = lambda i: st1(i) + ap1(i)

        def qkv(i, part):
            ref = (q_s, k_s, v_s)[part][i]
            for r0, c0, v in mm576(KQ, wa_s[part], ha_s[i % 3]):
                ref[r0:r0 + v.shape[0], c0:c0 + v.shape[1]] = v

        lane = lax.broadcasted_iota(jnp.int32, (8, 128), 1)
        NT_ = S // 128
        HW = W // 2
        back = lambda prev, cur, s: pltpu.roll(jnp.where(lane >= 128 - s, prev, cur), s, 1)
        ahead = lambda cur, nxt, s: pltpu.roll(jnp.where(lane >= s, cur, nxt), 128 - s, 1)
        tile = lambda refs, t, r0: refs[t // 4][r0:r0 + 8, t % 4 * 128:(t % 4 + 1) * 128]
        far, prob, lost = {}, {}, {}

        def qk(t):
            st = {}

            def f(g, d0):
                for d in range(d0, d0 + AD):
                    r0 = d * H + g * 8
                    qv, kv = tile(q_s, t, r0), tile(k_s, t, r0)
                    qa = ahead(qv, tile(q_s, min(t + 1, NT_ - 1), r0), HW * DIL)
                    kp = tile(k_s, max(t - 1, 0), r0)
                    ks = [kv] + [back(kp, kv, w * DIL) for w in range(1, HW)]
                    pr = [qv * kk for kk in ks] + [qa * kk for kk in ks]
                    st["l"] = pr if d == 0 else add(st["l"], pr)
                if d0 + AD == DH:
                    for w in range(HW):
                        far_s[t % 2, g, w] = st["l"][HW + w]
                    lg = st["l"][:HW] + [back(far_s[1 - t % 2, g, w] if t else b, b, HW * DIL) for w, b in enumerate(st["l"][HW:])]
                    lg = [l * (DH ** -0.5) for l in lg]
                    if t == 0:
                        lg = [jnp.where(lane >= w * DIL, lg[w], -1e9) for w in range(W)]
                    mx = functools.reduce(jnp.maximum, lg)
                    e = [jnp.exp(l - mx) for l in lg]
                    inv = 1.0 / functools.reduce(jnp.add, e)
                    pw = [a * inv for a in e]
                    if t == 0:
                        lost[g] = functools.reduce(jnp.add, [jnp.where(lane >= w * DIL, 0.0, a) for w, a in enumerate(pw)])
                        pw = [jnp.where(lane >= w * DIL, a, 0.0) for w, a in enumerate(pw)]
                    for w in range(W):
                        p_s[t, g, w] = pw[w]
                return st["l"][-1]
            return [(AC * AD, k_s[t // 4], P(f, g, d0)) for g in range(4) for d0 in range(0, DH, AD)]

        def pv(t):
            st = {}

            def f(g, d0):
                if d0 == 0:
                    st["p"] = [p_s[t + zero, g, w] for w in range(HW)]
                    st["a"] = [ahead(p_s[t + zero, g, w], p_s[min(t + 1, NT_ - 1) + zero, g, w], HW * DIL) for w in range(HW, W)]
                for d in range(d0, d0 + AD):
                    r0 = d * H + g * 8
                    vv = tile(v_s, t, r0)
                    vp = tile(v_s, max(t - 1, 0), r0)
                    vs = [vv] + [back(vp, vv, w * DIL) for w in range(1, HW)]
                    near = functools.reduce(jnp.add, [a * b for a, b in zip(st["p"], vs)])
                    part = functools.reduce(jnp.add, [a * b for a, b in zip(st["a"], vs)])
                    pp_s[t % 2, r0:r0 + 8] = part
                    if t:
                        y = back(pp_s[1 - t % 2, r0:r0 + 8], part, HW * DIL)
                    else:
                        v0 = jnp.where(lane == 0, vv, 0.0)
                        for sh in (1, 2, 4, 8):
                            v0 = v0 + pltpu.roll(v0, sh, 1)
                        y = back(jnp.zeros_like(part), part, HW * DIL) + lost.get(g, v0) * v0
                    o_s[r0:r0 + 8, t % 4 * 128:(t % 4 + 1) * 128] = near + y
                return o_s
            return [(AC * AD, v_s[t // 4], P(f, g, d0)) for g in range(4) for d0 in range(0, DH, AD)]

        def enc_o(i):
            return enc_act(KO, tiles(o_s, 0), oa_s, o_s, 3)

        def proj(i):
            for r0, c0, v in mm576(KO, wa_s[3], oa_s):
                m, n = v.shape
                xv = xs[r0:r0 + m, i * TM + c0:i * TM + c0 + n].astype(f32)
                for c in range(0, n, 128):
                    x1_s[i % 2][r0:r0 + m, c0 + c:c0 + c + 128] = xv[:, c:c + 128] + mcol(2, r0, m) * v[:, c:c + 128]

        def ln2(i):
            ps, out = norm(tiles(x1_s[i % 2], 0), x1_s[i % 2], 3, 4)

            def enc(r0, k):
                rows[k] = out(k * 128 + r0, 16)
                if k == 3:
                    for r, e in enumerate(encode(enc_a1, K1, lambda p, k: rows[k][p])):
                        h2_s[r, r0:r0 + 16] = e.astype(bf16)
                    return h2_s

            def tail():
                one = (lax.broadcasted_iota(jnp.int32, (DP - D, 128), 0) == 0).astype(f32)
                for t, v in enumerate(out(512, 64)):
                    hr_s[t] = pltpu.bitcast(jnp.concatenate([v, one], axis=0).astype(bf16).T, u32)

            def tr(rs):
                for r in rs:
                    he_s[r, 0:64] = pltpu.bitcast(ld(h2_s, (r,), 0, 128).T, u32)
                return he_s
            rows, order1 = {}, []
            for _ in decode(K1, lambda r: (order1.append(r), Sym())[1], lambda v: (lambda: v)):
                pass
            return (ps + [(32 + 105 * (k == 3), x1_s[i % 2], P(enc, r0, k)) for r0 in range(0, 128, 16) for k in range(4)]
                    + [(150, x1_s[i % 2], tail)] + [(200, h2_s, P(tr, order1[r:r + 7])) for r in range(0, 49, 7)])

        def prep_w(src, dst, enc1, kinds, rb, j, quads):
            blk = {}

            def f(r0, k, C):
                v = src[k * rb + r0:k * rb + r0 + 16, j * 512 + C * 256:j * 512 + C * 256 + 256].astype(f32)
                blk[k, 2 * C], blk[k, 2 * C + 1] = v[:, :128], v[:, 128:]
                if len(blk) == 16:
                    for r, e in enumerate(encode(enc1, kinds, lambda k, q: blk[k, q])):
                        dst[j, r, r0:r0 + 16] = e.astype(bf16)
                    blk.clear()
            return [(4 + 4 * so + no * ci, src, P(f, r0, 2 * R + (quads[0][2] ^ h), C)) for r0 in range(0, rb, 16)
                    for so, no, R, C in quads for h, ci in ((0, 4), (1, 11))]

        def prep_w1(j):
            def tail():
                brow = b1_ref[...].reshape(1, F).astype(f32)[:, j * 512:(j + 1) * 512]
                first = lax.broadcasted_iota(jnp.int32, (64, 512), 0) == 0
                v = jnp.concatenate([w1_s[512:D, j * 512:(j + 1) * 512].astype(f32), jnp.where(first, brow, 0.0)], axis=0)
                for q in range(4):
                    w1r[j, q] = v[:, q * 128:(q + 1) * 128].astype(bf16)
            return prep_w(w1_s, w1e, enc_b1, K1, 128, j, ((0, 1, 0, 0), (1, 1, 0, 1), (2, 3, 1, 1), (1, 2, 1, 0))) + [(80, w1_s, tail)]

        prep_w2 = lambda j: prep_w(w2_s, w2e, enc_a1, K2, 144, j, ((0, 1, 1, 1), (1, 1, 1, 0), (2, 3, 0, 0), (1, 2, 0, 1)))
        posts = {}

        def ffn1(i, j):
            n = i * NC + j
            zs = z_s[n % NZ]
            cnt = [0]

            def prod(r):
                cnt[0] += 1
                if n - 2 in posts and cnt[0] == DA:
                    join(posts[n - 2], DL)
                if HALF and cnt[0] == (DA + 24) % 49 + 1 and (n - 2 + (DA < 25), 0) in posts:
                    join(posts[n - 2 + (DA < 25), 0], DL)
                return mm(tied(he_s[r, 0:64]), ld(w1e, (j, r), 0, 128))

            for (p, q), v in decode(K1, prod, stash):
                zs[p % 2 * 2 + q % 2][p // 2 * 2 + q // 2, 0:128] = v + mm(pltpu.bitcast(hr_s[p], bf16), ld(w1r, (j, q), 0, 128))
            gv = {}

            def post(r0, Q, Pp, q, p):
                z = zs[p * 2 + q][Pp * 2 + Q, r0:r0 + 16]
                gv[2 * Q + q, 2 * Pp + p] = z + z * jnp.tanh(z * (C0 + C1 * (z * z)))
                if (Q, Pp, q, p) == (1, 0, 1, 0):
                    for r, e in enumerate(encode(enc_b1, K2, lambda q, p: gv[q, p])):
                        (g0, g1)[i % 2][j, r, r0:r0 + 16] = e.astype(bf16)
                    return (g0, g1)[i % 2][j + zero, 48, r0:r0 + 16].astype(f32)[0:8] if DL and r0 in (48, 112) else None
            wo_ = ((0, 1, 0, 0), (1, 1, 0, 1), (2, 3, 1, 1), (1, 2, 1, 0))
            ps = [(PB + 2 * so + no * (2 * si + ni), zs[p * 2 + q], P(post, r0, Q, Pp, q, p)) for r0 in range(0, 128, 16)
                  for so, no, Q, Pp in wo_ for si, ni, q, p in wo_]
            ps = [(sum(x[0] for x in ps[k:k + GR]), [x[1] for x in ps[k:k + GR]], P(lambda fs: [f() for f in fs][-1], [x[2] for x in ps[k:k + GR]]))
                  for k in range(0, len(ps), GR)]
            if HALF:
                posts[n, 0] = spawn(ps[:64 // GR], PT // 2)
                posts[n] = spawn(ps[64 // GR:], PT // 2, PT // 2)
            else:
                posts[n] = spawn(ps, PT)

        def out_copy(i, h):
            r0, m, c0, n = ((0, D, 0, TM), (0, D, 0, 256), (288, 288, 256, 256), (0, 288, 256, 256))[h]
            sl = (pl.ds(r0, m), pl.ds(i * TM + c0, n))
            return pltpu.make_async_copy(out_s.at[sl], o_hbm.at[sl], osem.at[i + h])

        order2 = []
        for _ in decode(K2, lambda r: (order2.append(r), Sym())[1], lambda v: (lambda: v)):
            pass

        class Ffn2:
            def __init__(self, i):
                self.i, self.res, self.n, self.done = i, {}, 0, {}
                self.seen, self.pre = [], {}
                self.probe = decode(K2, lambda r: (self.seen.append(r), Sym())[1], lambda v: (lambda: v))
                self.dec = decode(K2, lambda r: self.res.pop(r)(), P(stash, pool=1))
                self.nxt = next(self.probe)

            def part(self, r, js, acc):
                for j in js:
                    join(posts.get(self.i * NC + j, ()))
                    y = mm(tied(w2e.bitcast(u32)[j, r]), ld((g0, g1)[self.i % 2], (j, r), 0, 128), NT)
                    acc = y if acc is None else acc + y
                return acc

            def early(self, n, k):
                for r in order2[:n]:
                    self.pre[r] = (k, stash(self.part(r, range(k), None)))

            def upto(self, n):
                i = self.i
                while True:
                    while self.nxt is not None and len(self.seen) <= self.n:
                        (r, c), v = next(self.dec)
                        self.nxt = next(self.probe, None)
                        rs = slice(r * 144, (r + 1) * 144)
                        y = x1_s[i % 2][rs, c * 128:(c + 1) * 128] + mcol(0, r * 144, 144) + mcol(1, r * 144, 144) * v
                        out_s[rs, i * TM + c * 128:i * TM + (c + 1) * 128] = y.astype(bf16)
                    if self.n >= n:
                        break
                    r = order2[self.n]; self.n += 1
                    k, a = self.pre.pop(r, (0, lambda: None))
                    self.res[r] = stash(self.part(r, range(k, NC), a()), 1)

        def gate2():
            def f():
                gb = mcol(5, 0, D)
                modc[0:D, :] = gb * col_of_row(pad0(b2_ref[...].reshape(1, D).astype(f32), DP, 1))[:D]
                modc[D:2 * D, :] = gb * 0.5
            return [(150, modc, f)]

        f2 = [Ffn2(i) for i in range(NB)]
        outs = []

        def out(i, h):
            out_copy(i, h).start(); outs.append((i, h))

        def bar():
            pl.semaphore_signal(bsem, 1)
            pl.semaphore_wait(bsem, 1)

        def stream(names):
            dst = dict(x=(xs, 512), wo=(wo_s, 640), wm=(wm_s, 384), w1=(w1_s, 512), w2=(w2_s, 512))
            ps = [(dst[n[:-1]][1], dst[n[:-1]][0], cps[n[:-1]][int(n[-1])].start) for n in names]
            spawn(ps, sum(p[0] for p in ps) * DR)

        acts = dict(bar=bar, mm=mod_mm, init=init, st1=st1, ap1=ap1, pq=prep_wqkv, mod=mod_cols, ln1=ln1, qkv=qkv, qk=qk, pv=pv, pwo=prep_wo, proj=proj, ln2=ln2, eo=enc_o,
                    pw1=prep_w1, pw2=prep_w2, f1=ffn1, f2=lambda i, n: f2[i].upto(n), gate=gate2, e2=lambda i, n, k: f2[i].early(n, k), out=out)
        named = []
        stack = contextlib.ExitStack()
        for line in (PROG if order is None else order if isinstance(order, str) else "\n".join(l if ">" not in l else "! bar" for l in PROG.strip().split("\n")[order[0]:order[1]])).replace(";", "\n").split("\n"):
            if ">" in line:
                if ">>" not in line:
                    for q in named:
                        join(q)
                stack.close()
                dma(*[x.strip() for x in line.replace(">>", ">").split(">")])
                continue
            toks = line.replace("+", " ").split()
            if toks and toks[0] == "stream":
                stream(toks[1:])
                continue
            dur = [int(x) for x in toks.pop(0)[1:].split("@")] if toks and toks[0][0] == "~" else None
            pend = []
            if SC and dur is None:
                stack.close(); stack.enter_context(scope("L_" + "_".join(toks)))
            for a in toks:
                if a[0] == "!":
                    for q in (jobs if a == "!!" else named if a == "!" else [named[-1 - int(a[1:])]]):
                        join(q, TIE)
                    continue
                a = a.split(".")
                rng = [int(x) for x in a[-1].split("-")] if len(a) > 1 else []
                calls = ([[int(x) for x in a[1:-1]] + [v] for v in range(rng[0], rng[1] + 1)] if len(rng) == 2
                         else [[int(x) for x in a[1:]]])
                for args in calls:
                    ps = acts[a[0]](*args) or []
                    if dur is None:
                        join(collections.deque((0, p) for p in ps))
                    pend += ps
            if dur is not None:
                named.append(spawn(pend, *[x * TS for x in dur]))
        for q in jobs:
            join(q)
        stack.close()
        for ih in outs:
            out_copy(*ih).wait()
        if order:
            for r in jax.tree.leaves([q_s, k_s, v_s, o_s, x1_s, he_s, p_s, hr_s, w1e, w2e, g0, g1, out_s, wa_s, ha_s, oa_s]):
                ix = (0,) * (len(r.shape) - 2) + (pl.ds(pl.multiple_of(zero * 8, 8), 8), slice(0, 128))
                out_s[0:8, 0:128] = out_s[0:8, 0:128] + r[ix].astype(jnp.int32 if r.dtype == u32 else f32).astype(bf16)
            c = out_copy(0, 0); c.start(); c.wait()

    @jax.jit
    def fn(A_x, A_wqkv, A_wo, B_x, B_w1, B_b1, B_w2, B_b2, c, w_mod):
        vm = pl.BlockSpec(memory_space=pltpu.VMEM)
        hb = pl.BlockSpec(memory_space=pl.ANY)
        V = pltpu.VMEM
        E = D + 16
        blk = [V((E, TM), f32)] * NB
        blk2 = blk[:2]
        out = pl.pallas_call(
            kernel,
            out_shape=jax.ShapeDtypeStruct((D, S), bf16),
            in_specs=[hb, hb, hb, hb, hb, hb, hb, hb, hb],
            out_specs=hb,
            scratch_shapes=[
                V((1, D), bf16), V((F,), bf16), V((D,), bf16), V((E, S), bf16), V((E, 3 * D), bf16), V((E, D), bf16), V((E, F), bf16), V((E, F), bf16),
                V((E, 6 * D), bf16), V((D, S), bf16), V((5, 3 * D // 2 + 16, 128), u32), V((5, E, 128), f32), V((5, E, 128), f32),
                V((48, 2 * D), f32), V((6 * D + 16, 128), f32), blk, blk, blk, V((E, TM), f32), V((2, D, 128), f32), V((2, 4, 4, 8, 128), f32), V((16, 4, 8, 8, 128), f32), blk2,
                V((49, 144, 128), bf16), V((49, 80, 128), u32), V((4, 64, 128), u32),
                V((NC, 49, 128, 128), bf16), V((NC, 4, 128, 128), bf16), V((NC, 49, 144, 128), bf16),
                V((NC, 49, 128, 128), bf16), V((NC, 49, 128, 128), bf16),
                [[V((4, 144, 128), f32)] * 4] * NZ, V((2 * NS, 144, 128), f32),
                [wshape(k) for k in (KQ, KQ, KQ, KO)], [ashape(KQ)] * 3, ashape(KO),
                pltpu.SemaphoreType.DMA((38,)), pltpu.SemaphoreType.DMA((2 * NB,)), pltpu.SemaphoreType.REGULAR, pltpu.SemaphoreType.REGULAR,
            ],
            compiler_params=pltpu.CompilerParams(vmem_limit_bytes=127 * 2**20, flags=flags, disable_bounds_checks=NOB),
        )(c, B_b1, B_b2, A_x.reshape(S, D).T, A_wqkv, A_wo, B_w1, B_w2.T, w_mod)
        return out.T.reshape(1, S, D)
    return fn


_impl = build()


@jax.jit
def pallas_adaLN_cond__sliding_local_dilated__dense_activation_gelu__prompt_kernel(
    A_x, A_wqkv, A_wo, B_x, B_w1, B_b1, B_w2, B_b2, c, w_mod):
    return _impl(A_x, A_wqkv, A_wo, B_x, B_w1, B_b1, B_w2, B_b2, c, w_mod)
```

```python
import collections
import functools

import numpy as np
import jax
import jax.numpy as jnp
from jax import lax
import jax.experimental.pallas as pl
import jax.experimental.pallas.tpu as pltpu

S, D, F = 2048, 576, 4608
H, DH, W, DIL = 32, 18, 8, 2
EPS = 1e-5
TM = 512
NB, NT, NC = S // TM, S // 128, F // 512
DQ = D // 4
KM = 112
E = D + 16
C0 = float(np.sqrt(2.0 / np.pi))
GA = float(np.cbrt(C0 * 0.044715))
f32, bf16, u32 = jnp.float32, jnp.bfloat16, jnp.uint32
P = functools.partial


def tmap(f, *xs):
    if isinstance(xs[0], (list, tuple)):
        return [tmap(f, *ys) for ys in zip(*xs)]
    return f(*xs)


add = P(tmap, lambda x, y: x + y)
sub = P(tmap, lambda x, y: x - y)
total = P(functools.reduce, lambda x, y: x + y)


def left_sums(a11, a12, a21, a22):
    s1 = add(a21, a22); s2 = sub(s1, a11)
    return [a11, a12, sub(a12, s2), a22, s1, s2, sub(a11, a21)]


def right_sums(b11, b12, b21, b22):
    t1 = sub(b12, b11); t2 = sub(b22, t1)
    return [b11, b21, b22, sub(t2, b21), t1, t2, sub(b22, b12)]


def encode(sums, blk):
    quad = lambda R, C: [blk(2 * R + r, 2 * C + c) for r in range(2) for c in range(2)]
    return [e for lv in sums(quad(0, 0), quad(0, 1), quad(1, 0), quad(1, 1)) for e in sums(*lv)]


strassen_left = lambda a, b, c, d: [a + d, c + d, a, d, a + b, c - a, b - d]
strassen_right = lambda a, b, c, d: [a + d, a, b - d, c - a, d, a + b, c + d]
STEPS = (0, 1, 5, 6, 3, 4, 2)
ORDER = [7 * a + b for a in STEPS for b in STEPS]


def combine(state, m, v, keep):
    if m == 0:
        state["m0"] = keep(v, 0)
    elif m == 1:
        return [(0, state["m0"]() + v)]
    elif m == 5:
        state["u2"] = keep(state["m0"]() + v, 1)
    elif m == 6:
        state["u3"] = keep(state["u2"]() + v, 0)
    elif m == 3:
        return [(2, state["u3"]() - v)]
    elif m == 4:
        state["u4"] = keep(state["u2"]() + v, 0)
        return [(3, state["u3"]() + v)]
    else:
        return [(1, state["u4"]() + v)]
    return []


def decoder(stash):
    inner, outer = {}, [{}, {}, {}, {}]

    def feed(r, v):
        return [((2 * (Q // 2) + q // 2, 2 * (Q % 2) + q % 2), c)
                for q, m in combine(inner, r % 7, v, lambda x, far: stash(x) if far else (lambda: x))
                for Q, c in combine(outer[q], r // 7, m, lambda x, far: stash(x))]
    return feed


ROWS = {0: (1, 1), 1: (1, 0), 2: (1, 0), 3: (0, 1), 4: (1, 1), 6: (0, 1)}
SLICES = [(u, v) for u in ((1, 0), (0, 1), (1, 1)) for v in ((1, 0), (0, 1), (1, 1))]
NO_RIDER = [r for r in range(49) if 5 in divmod(r, 7)]
riders = lambda s: [(a, b) for a in ROWS for b in ROWS if (ROWS[a], ROWS[b]) == SLICES[s]]
col_coef = lambda m, w1, w2: w1 if m in (0, 1) else w2 if m in (2, 6) else sub(w2, w1)

PROGRAM = """
> s0 x0 wq0 wm0 wm1 wm2
pin
s0 x0 >
st1.0.0.2
wq0 > x4
pq.0
wm0 wm1 > wq1
mod.0-1 col.0-1
wm2 > wq2 x1
mod.2 col.2 ap1.0.0 qkv.0.0.0.1
x4 > s1 s2
~600 st1.0.2.2 ap1.0.2
qkv.0.0.1.2
wq1 >
stream x2 x3 wo0 wm3 wm4 wm5 wm6 wm7 wm8 w10 w11 w12 w13 w14 w15 w16 w17 w18 w20 w21 w22 w23 w24 w25 w26 w27 w28
~1200 pq.1
qkv.0.0.2.4
wq2 >
~1200 pq.2
qkv.0.1.0.2
x1 >
~3800 ln1.1
~3600 qk.0-1
qkv.0.1.2.4 qkv.0.2
x2 >
~4900 ln1.2
~4500 qk.2-3 pv.0
qkv.1.0-1
s1 s2 x3 wo0 wm3 wm4 wm5 wm6 wm7 wm8 >
~6200 qk.4-6 pv.1-3
~3700@6300 pwo col.3-8
~6000 st1.3
~4000@6100 ap1.3
mod.3-8 qkv.1.2 qkv.2.0-2
w10 w11 w12 w13 w14 w15 w16 w17 w18 >
~2600 pw1.0-2
proj.0
~7600 pw1.3-8
~7500 ln2.0
qkv.3.0-2
w20 w21 w22 w23 w24 w25 >
~1900 pw2.0-1
~11000@1950 pw2.2-4
up.0.0-8
w26 w27 w28 >
down.0.40.5
~3800@3200 pw2.5-8
~1200@2000 qk.7
go.200 !! bar
~200 gate
~4300 qk.8 pv.4-7
go.128 ! proj.1
~3800 ln2.1
go.113 ! bar
~1800 qk.9
up.1.0-8 down.1.16.5 go.63
~8400@200 qk.10-12 pv.8-11
go.251 ! proj.2
~4300 ln2.2
go.127 ! bar
~1800 qk.13
up.2.0-8 down.2.16.5 go.63
~8000@200 qk.14-15 pv.12-15
go.239 ! proj.3
~4700 ln2.3
go.139 ! bar
up.3.0-8 down.3.49.5
go.441
"""


LINES = PROGRAM.strip().split("\n")
WAITS = [l.split(">")[0].split() for l in LINES if ">" in l and l.split(">")[0].strip()]
SEM_OF = {n: k for k, names in enumerate(WAITS) for n in names}
PT, PB, GAP, TC, DR = 2000, 12, 150, 170, 2.25
NS = 40


def kernel(c_hbm, b1_hbm, b2_hbm, x_hbm, wqkv_hbm, wo_hbm, w1_hbm, w2_hbm, wm_hbm, o_hbm,
           c_s, b1_s, b2_s, x_s, wqkv_s, wo_s, w1_s, w2_s, wm_s, out_s, wqt_s, wof_s, wot_s, row_s, col_s,
           q_s, k_s, v_s, o_s, part_s, far_s, p_s, x1_s, h2_s, he_s, w1e_s, w1r_s, w2e_s, g_s, acc_s, z_s,
           tmp_s, wa_s, h1_s, ob_s, sems, osem, zsem, bsem):
    def copy(name):
        kind, k = name[:-1], int(name[-1])
        sem = sems.at[SEM_OF[name]]
        if kind == "s":
            return pltpu.make_async_copy(*((c_hbm, c_s), (b1_hbm, b1_s), (b2_hbm, b2_s))[k], sem)
        if kind == "wo":
            return pltpu.make_async_copy(wo_hbm, wo_s.at[pl.ds(0, D)], sem)
        src, dst, cols = {
            "wq": (wqkv_hbm, wqkv_s, ((0, 640), (640, 512), (1152, 576))[k % 3]),
            "x": (x_hbm, x_s, ((0, 256), (512, TM), (1024, TM), (1536, TM), (256, 256))[k % 5]),
            "wm": (wm_hbm, wm_s, (k * 384, 384)),
            "w1": (w1_hbm, w1_s, (k * 512, 512)), "w2": (w2_hbm, w2_s, (k * 512, 512))}[kind]
        return pltpu.make_async_copy(src.at[:, pl.ds(*cols)], dst.at[pl.ds(0, D), pl.ds(*cols)], sem)

    zero = pl.semaphore_read(zsem)
    clock = dict(t=0.0, n=0, post=0.0)
    jobs = []

    def spawn(pieces, dur, delay=0):
        t, scale, q = clock["t"] + delay, dur / sum(p[0] for p in pieces), collections.deque()
        for p in pieces:
            q.append((t, p)); t += scale * p[0]
        jobs.append(q)
        return q

    def finish(q):
        while q:
            q.popleft()[1][2]()

    def mm(a, b, rhs_axis=0):
        y = lax.dot_general(a, b, (((1,), (rhs_axis,)), ((), ())), preferred_element_type=f32)
        m, t0 = a.shape[0], clock["t"]
        while clock["n"] % 4 == 0:
            due = [q for q in jobs if q and q[0][0] < t0 + m]
            if not due:
                break
            t, (_, ref, fn) = min(due, key=lambda q: q[0][0]).popleft()
            if ref is not None:
                r = int(max(t - t0, 0.0)) // 8 * 8
                spare = pl.ds(pl.multiple_of(ref.shape[-2] - 16 + zero * 16, 16), 8)
                ref[(0,) * (len(ref.shape) - 2) + (spare, slice(0, 128))] = (
                    pltpu.bitcast(y[r:r + 8], u32) if ref.dtype == u32 else y[r:r + 8].astype(ref.dtype))
            fn()
        clock["t"] += m / 4; clock["n"] += 1
        return y

    def barrier():
        pl.semaphore_signal(bsem, 1)
        pl.semaphore_wait(bsem, 1)

    def pin():
        for r in jax.tree.leaves([tmp_s, part_s, far_s, he_s, g_s, acc_s, w1e_s, w1r_s, w2e_s, wa_s, h1_s, ob_s, o_s]):
            r[(zero,) + (0,) * (len(r.shape) - 3) + (slice(0, 8), slice(0, 128))] = jnp.zeros((8, 128), r.dtype)
        for r in h1_s + [ob_s]:
            r[:, 14:16, 64:128] = jnp.zeros((2, 2, 64, 128), bf16)
        for r in NO_RIDER:
            h2_s[r, KM:128] = jnp.zeros((16, 128), bf16)
            w1e_s[:, r, KM:128] = jnp.zeros((NC, 16, 128), bf16)
        row, a, left = lax.broadcasted_iota(jnp.int32, (16, 128), 0), 0.0, GA
        for k in range(3):
            piece = float(np.asarray(left, bf16)); left -= piece
            a = jnp.where(row == k, piece, a)
        for m, n in riders(8):
            h2_s[7 * m + n, KM:128] = a.astype(bf16)

    slot = [0, 0]

    def stash(v, pool):
        k = pool * NS + slot[pool] % NS; slot[pool] += 1
        tmp_s[k, 0:v.shape[0]] = v
        return lambda: tmp_s[k, 0:v.shape[0]]

    def operand(ref, ix, r0, n):
        return pltpu.bitcast(ref.bitcast(u32)[ix + (slice(r0 // 2, (r0 + n) // 2),)], bf16)

    def pad0(v, n, axis):
        shape = list(v.shape); shape[axis] = n - shape[axis]
        return jnp.concatenate([v, jnp.zeros(shape, v.dtype)], axis=axis) if shape[axis] else v

    fold = lambda v: total([v[r:r + 8] for r in range(0, v.shape[0], 8)])
    col = lambda i, r0, n: col_s[i * D + r0:i * D + r0 + n, :]

    def mod_rows(k):
        cv = c_s[...].astype(f32)
        act = jnp.broadcast_to(cv * jax.nn.sigmoid(cv), (16, D)).astype(bf16)
        y = jnp.dot(act, wm_s[0:D, k * 384:(k + 1) * 384], preferred_element_type=f32)[0:8]
        ch = lax.broadcasted_iota(jnp.int32, y.shape, 1) + k * 384
        scale = ((ch >= D) & (ch < 2 * D)) | ((ch >= 4 * D) & (ch < 5 * D))
        row_s[8 * k:8 * k + 8] = jnp.where(scale, y + 1.0, y) * jnp.where((ch >= 3 * D) & (ch < 5 * D), GA, 1.0)

    def mod_cols(k):
        def f(t):
            row = row_s[8 * k:8 * k + 8, t * 128:(t + 1) * 128]
            col_s[(3 * k + t) * 128:(3 * k + t + 1) * 128, :] = jnp.concatenate([row] * 16, axis=0).T
        return [(60, row_s, P(f, t)) for t in range(3)]

    def gate():
        def f():
            b2 = pad0(b2_s[...].reshape(1, D).astype(f32), 640, 1)
            col_s[0:D, :] = col(5, 0, D) * jnp.broadcast_to(b2, (128, 640)).T[:D]
            col_s[D:2 * D, :] = col(5, 0, D) * (0.5 / GA)
        return [(150, col_s, f)]

    def put_weight(i, load, src):
        def f(r0):
            for k in range(2):
                for m, e in enumerate(strassen_left(*[load(c + k, r + r0) for r in (0, D // 2) for c in (0, 2)])):
                    wa_s[i][2 * m + k, r0:r0 + 16] = e.astype(bf16)
                wa_s[i][14 + k, r0:r0 + 16] = load(4, k * (D // 2) + r0).astype(bf16)
        return [(50, src, P(f, r0)) for r0 in range(0, D // 2, 16)]

    def put_input(dst, pair, r0, rows):
        if r0 < 512:
            for m, e in enumerate(strassen_right(*rows(r0 - 256), *rows(r0))):
                dst[pair, 2 * m + r0 // 128 - 2, r0 % 128:r0 % 128 + 16] = e.astype(bf16)
        else:
            for m, e in enumerate(rows(r0)):
                dst[pair, 14 + m, r0 - 512:r0 - 496] = e.astype(bf16)

    def prep_wqkv(i):
        c0, c1 = ((0, 640), (640, 1152), (1152, 3 * D))[i]

        def tr(k):
            blk = pad0(wqkv_s[k * 128:min(D, (k + 1) * 128), c0:c1], 128, 0)
            wqt_s[k, c0 // 2:c1 // 2] = pltpu.bitcast(blk.T, u32)

        def load(k, r0):
            d, h0 = divmod(r0, H)
            u = wqt_s[k, pl.ds(i * (D // 2) + h0 * (DH // 2) + d // 2, 16, stride=DH // 2), :]
            return pltpu.bitcast(u & np.uint32(0xFFFF0000) if d % 2 else u << 16, f32)
        return [(100, wqkv_s, P(tr, k)) for k in range(5)] + put_weight(i, load, wqt_s)

    def prep_wo():
        def widen(n, r0):
            wof_s[n, r0:r0 + DQ] = pad0(wo_s[r0:r0 + DQ, n * 128:min(D, (n + 1) * 128)].astype(f32), 128, 1)

        def tr(n, k):
            rows = [wof_s[n, pl.ds(d, H, stride=DH), :] for d in range(4 * k, min(DH, 4 * k + 4))]
            m = min(128, D - n * 128)
            wot_s[k, n * 128:n * 128 + m] = pad0(jnp.concatenate(rows, axis=0), 128, 0).T[:m]
        return ([(40, wo_s, P(widen, n, r0)) for n in range(5) for r0 in range(0, D, DQ)]
                + [(60, wof_s, P(tr, n, k)) for n in range(5) for k in range(5)]
                + put_weight(3, lambda k, r0: wot_s[k, r0:r0 + 16], wot_s))

    def project(w, act, put, n0, n1):
        for pair, r0 in [(pair, r0) for pair in range(2) for r0 in (0, DQ)][n0:n1]:
            one = lambda a, b: mm(operand(w, (a,), r0, DQ), operand(act, (pair, b), 0, 128))
            m = lambda k: one(2 * k, 2 * k) + one(2 * k + 1, 2 * k + 1)
            out = lambda R, C, y: put(R * (D // 2) + r0, (2 * pair + C) * 128, y + one(14 + R, 14 + C))
            m0 = m(0)
            c11, c22 = stash(m0 + m(6), 0), stash(m0 + m(5), 0)
            m1, m3 = m(1), m(3)
            c11, c22 = stash(c11() + m3, 0), stash(c22() - m1, 0)
            out(1, 0, m1 + m3)
            m2 = m(2)
            out(1, 1, c22() + m2)
            m4 = m(4)
            out(0, 1, m2 + m4)
            out(0, 0, c11() - m4)

    def norm(ref, c0, nt, shift, scale, sums=None):
        LR = 8 if nt == 4 else 32
        mean = lambda a: jnp.sum(a, axis=0, keepdims=True) * (1.0 / D)
        st = {"m": [mean(a) for a in sums]} if sums else {}

        def load(r0, n):
            v = ref[r0:r0 + n, c0:c0 + nt * 128].astype(f32)
            return [v[:, t * 128:(t + 1) * 128] for t in range(nt)]

        def first(r0):
            y = [fold(t) for t in load(r0, LR)]
            st["a"] = add(st["a"], y) if r0 else y
            if r0 == D - LR:
                st["m"] = [mean(a) for a in st["a"]]

        def second(r0):
            y = [fold((t - m) * (t - m)) for t, m in zip(load(r0, LR), st["m"])]
            st["a"] = add(st["a"], y) if r0 else y
            if r0 == D - LR:
                st["r"] = [lax.rsqrt(mean(a) + EPS) for a in st["a"]]

        def apply(r0, which):
            v, sc, sh = load(r0, 16), col(scale, r0, 16), col(shift, r0, 16)
            return [((v[t] - st["m"][t]) * st["r"][t]) * sc + sh for t in which]
        gap = [(GAP, None, lambda: None)]
        return ([(LR, ref, P(first, r0)) for r0 in range(0, 0 if sums else D, LR)] + gap
                + [(2 * LR, ref, P(second, r0)) for r0 in range(0, D, LR)] + gap), apply

    norm1 = {}

    def ln1_stats(i, t0=0, nt=4):
        pieces, apply = norm(x_s, i * TM + t0 * 128, nt, 0, 1)
        norm1[i, t0] = (apply, nt)
        return pieces

    def ln1_apply(i, t0=0):
        apply, nt = norm1[i, t0]
        return [(57 if r0 < 512 else 22, x_s, P(put_input, h1_s[i % 3], (t0 + t) // 2, r0, P(apply, which=(t, t + 1))))
                for t in range(0, nt, 2) for r0 in range(256, D, 16)]

    def qkv(i, part, n0=0, n1=4):
        def put(r0, c0, y):
            (q_s, k_s, v_s)[part][i][r0:r0 + DQ, c0:c0 + 128] = y
        project(wa_s[part], h1_s[i % 3], put, n0, n1)

    HW = W // 2
    lane = lax.broadcasted_iota(jnp.int32, (8, 128), 1)
    back = lambda prev, cur, s: pltpu.roll(jnp.where(lane >= 128 - s, prev, cur), s, 1)
    ahead = lambda cur, nxt, s: pltpu.roll(jnp.where(lane >= s, cur, nxt), 128 - s, 1)
    tile = lambda refs, t, r0: refs[t // 4][r0:r0 + 8, t % 4 * 128:(t % 4 + 1) * 128]
    masked = {}

    def shifts(refs, t, r0):
        prev, cur = tile(refs, max(t - 1, 0), r0), tile(refs, t, r0)
        return [cur] + [back(prev, cur, w * DIL) for w in range(1, HW)]

    def scores(t):
        st = {}

        def f(g, d):
            r0 = d * H + g * 8
            q = tile(q_s, t, r0)
            qa = ahead(q, tile(q_s, min(t + 1, NT - 1), r0), HW * DIL)
            ks = shifts(k_s, t, r0)
            y = [q * k for k in ks] + [qa * k for k in ks]
            st["l"] = add(st["l"], y) if d else y
            if d == DH - 1:
                for w in range(HW):
                    far_s[t % 2, g, w] = st["l"][HW + w]
                lg = st["l"][:HW] + [back(far_s[1 - t % 2, g, w] if t else a, a, HW * DIL)
                                     for w, a in enumerate(st["l"][HW:])]
                lg = [a * (DH ** -0.5) for a in lg]
                if t == 0:
                    lg = [jnp.where(lane >= w * DIL, a, -1e9) for w, a in enumerate(lg)]
                top = functools.reduce(jnp.maximum, lg)
                e = [jnp.exp(a - top) for a in lg]
                inv = 1.0 / total(e)
                p = [a * inv for a in e]
                if t == 0:
                    masked[g] = total([jnp.where(lane >= w * DIL, 0.0, a) for w, a in enumerate(p)])
                    p = [jnp.where(lane >= w * DIL, a, 0.0) for w, a in enumerate(p)]
                for w in range(W):
                    p_s[t, g, w] = p[w]
        return [(24, k_s[t // 4], P(f, g, d)) for g in range(4) for d in range(DH)]

    def mixing(t):
        st = {}

        def f(g, d):
            if d == 0:
                st["p"] = [p_s[t + zero, g, w] for w in range(HW)]
                st["a"] = [ahead(p_s[t + zero, g, w], p_s[min(t + 1, NT - 1) + zero, g, w], HW * DIL)
                           for w in range(HW, W)]
            r0 = d * H + g * 8
            vs = shifts(v_s, t, r0)
            far = total([p * v for p, v in zip(st["a"], vs)])
            part_s[t % 2, r0:r0 + 8] = far
            y = total([p * v for p, v in zip(st["p"], vs)])
            if t:
                y = y + back(part_s[1 - t % 2, r0:r0 + 8], far, HW * DIL)
            else:
                v0 = jnp.where(lane == 0, vs[0], 0.0)
                for s in (1, 2, 4, 8):
                    v0 = v0 + pltpu.roll(v0, s, 1)
                y = y + back(jnp.zeros_like(far), far, HW * DIL) + masked[g] * v0
            if t % 2 and g % 2 and r0 > 256:
                last = jnp.concatenate([o_s[1, r0 - 8:r0], y], axis=0)
                put_input(ob_s, t % 4 // 2, r0 - 8,
                          lambda r: (o_s[0, r:r + 16], last if r == r0 - 8 else o_s[1, r:r + 16]))
            else:
                o_s[t % 2, r0:r0 + 8] = y
        return [((24 if t else 36) + 14 * (t % 2 * g % 2 * d >= 8), v_s[t // 4], P(f, g, d)) for g in range(4) for d in range(DH)]

    sums = {}

    def out_proj(i):
        def put(r0, c0, y):
            x1 = x_s[r0:r0 + DQ, i * TM + c0:i * TM + c0 + 128].astype(f32) + col(2, r0, DQ) * y
            x1_s[i % 2][r0:r0 + DQ, c0:c0 + 128] = x1
            sums[i, c0] = sums[i, c0] + fold(x1) if (i, c0) in sums else fold(x1)
        project(wa_s[3], ob_s, put, 0, 4)

    def ln2(i):
        src = x1_s[i % 2]
        pieces, apply = norm(src, 0, 4, 3, 4, [sums[i, c] for c in range(0, TM, 128)])
        blk = {}

        def main(r0, R, C):
            for k in range(2 * C, 2 * C + 2):
                blk[2 * R, k], blk[2 * R + 1, k] = apply(k * KM + r0, (2 * R, 2 * R + 1))
            if len(blk) == 16:
                for r, e in enumerate(encode(left_sums, lambda p, k: blk[p, k])):
                    h2_s[r, r0:r0 + 16] = e.astype(bf16)
                blk.clear()

        def rest(s):
            h = apply(4 * KM + 16 * s, range(4))
            rho = [x * y for x in SLICES[s][0] for y in SLICES[s][1]]
            a = total(h) if sum(rho) == 1 else total(h) * (1.0 / sum(rho))
            for p in range(4):
                h2_s[49 + p, 16 * s:16 * s + 16] = (h[p] - a if rho[p] else h[p]).astype(bf16)
            for m, n in riders(s):
                h2_s[7 * m + n, KM:128] = a.astype(bf16)

        def tr(rs):
            for r in rs:
                he_s[r] = pltpu.bitcast(operand(h2_s, (r,), 0, 128).T, u32)
        return (pieces + [(32 + c, src, P(main, r0, R, C)) for r0 in range(0, KM, 16)
                          for c, R, C in ((15, 1, 1), (23, 1, 0), (61, 0, 0), (38, 0, 1))]
                + [(50, src, P(rest, s)) for s in range(8)] + [(TC, h2_s, P(tr, range(49, 53)))]
                + [(TC, h2_s, P(tr, ORDER[r:r + 7])) for r in range(0, 49, 7)])

    def weight_sums(src, dst, sums_, rb, j, quads):
        blk = {}

        def f(r0, k, C):
            v = src[k * rb + r0:k * rb + r0 + 16, j * 512 + C * 256:j * 512 + C * 256 + 256].astype(f32)
            blk[k, 2 * C], blk[k, 2 * C + 1] = v[:, :128], v[:, 128:]
            if len(blk) == 16:
                for r, e in enumerate(encode(sums_, lambda k, q: blk[k, q])):
                    dst[j, r, r0:r0 + 16] = e.astype(bf16)
                blk.clear()
        return [(4 + 4 * a + n * c, src, P(f, r0, 2 * R + (quads[0][0] ^ h), C)) for r0 in range(0, rb, 16)
                for (a, n), (R, C) in zip(((0, 1), (1, 1), (2, 3), (1, 2)), quads) for h, c in ((0, 4), (1, 11))]

    def prep_w1(j):
        def rest(s):
            if s < 8:
                v = w1_s[4 * KM + 16 * s:4 * KM + 16 * s + 16, j * 512:(j + 1) * 512].astype(f32)
            else:
                b1 = b1_s[...].reshape(1, F).astype(f32)[:, j * 512:(j + 1) * 512]
                v = jnp.where(lax.broadcasted_iota(jnp.int32, (16, 512), 0) < 3, b1, 0.0)
            w = [v[:, q * 128:(q + 1) * 128] for q in range(4)]
            for q in range(4 if s < 8 else 0):
                w1r_s[j, q, 16 * s:16 * s + 16] = w[q].astype(bf16)
            for m, n in riders(s):
                w1e_s[j, 7 * m + n, KM:128] = col_coef(n, *col_coef(m, w[:2], w[2:])).astype(bf16)
        return (weight_sums(w1_s, w1e_s, right_sums, KM, j, ((0, 0), (0, 1), (1, 1), (1, 0)))
                + [(24, w1_s, P(rest, s)) for s in range(9)])

    prep_w2 = lambda j: weight_sums(w2_s, w2e_s, left_sums, DQ, j, ((1, 1), (1, 0), (0, 0), (0, 1)))
    gelus = {}

    def mlp_up(i, j):
        feed, seen, g = decoder(P(stash, pool=0)), {}, {}
        for r in ORDER:
            for (p, q), v in feed(r, mm(pltpu.bitcast(he_s[r], bf16), operand(w1e_s, (j, r), 0, 128))):
                k, tot = seen.get(q, (0, None))
                if k < 3:
                    y = mm(pltpu.bitcast(he_s[49 + p], bf16), operand(w1r_s, (j, q), 0, 128))
                    seen[q] = (k + 1, stash(tot() + y if k else y, 0))
                z_s[j][p % 2 * 2 + q % 2][p // 2 * 2 + q // 2, 0:128] = v + y if k < 3 else v - tot()

        def f(r0, Q, R, q, p):
            z = z_s[j][p * 2 + q][R * 2 + Q, r0:r0 + 16]
            g[2 * Q + q, 2 * R + p] = z + z * jnp.tanh(z * (C0 / GA + z * z))
            if len(g) == 16:
                for r, e in enumerate(encode(right_sums, lambda q, p: g[q, p])):
                    g_s[j][r, r0:r0 + 16] = e.astype(bf16)
                g.clear()
        walk = ((0, 1, 0, 0), (1, 1, 0, 1), (2, 3, 1, 1), (1, 2, 1, 0))
        lag = max(0.0, clock["post"] - clock["t"])
        gelus[j] = spawn([(PB + 2 * a + n * (2 * b + m), z_s[j][p * 2 + q], P(f, r0, Q, R, q, p))
                          for r0 in range(0, 128, 16) for a, n, Q, R in walk for b, m, q, p in walk], PT, lag)
        clock["post"] = clock["t"] + lag + PT

    passes, sent = collections.deque(), []

    def send(i, r0, m, c0, n):
        where = (pl.ds(r0, m), pl.ds(i * TM + c0, n))
        sent.append(pltpu.make_async_copy(out_s.at[where], o_hbm.at[where], osem))
        sent[-1].start()

    def mlp_down(i, *stages):
        feed, st, done = decoder(P(stash, pool=1)), {}, [0] * 49

        def f(r, j, j0, j1):
            finish(gelus[j])
            y = mm(operand(w2e_s, (j, r), 0, DQ), operand(g_s[j], (r,), 0, 128), 1)
            st["a"] = y if j == 0 else (acc_s[r] if j == j0 else st["a"]) + y
            if j == j1 - 1:
                acc_s[r] = st["a"]
            if j == NC - 1:
                for (d, c), v in feed(r, acc_s[r]):
                    x1 = x1_s[i % 2][d * DQ:(d + 1) * DQ, c * 128:(c + 1) * 128]
                    out_s[d * DQ:(d + 1) * DQ, i * TM + c * 128:i * TM + (c + 1) * 128] = (
                        x1 + col(0, d * DQ, DQ) + col(1, d * DQ, DQ) * v).astype(bf16)
                if i < NB - 1 and r == ORDER[-1]:
                    send(i, 0, D, 0, TM)
                if i == NB - 1 and r == ORDER[-8]:
                    send(i, 0, D, 0, 256); send(i, D // 2, D // 2, 256, 256)
                if i == NB - 1 and r == ORDER[-2]:
                    send(i, 0, D // 2, 256, 128); send(i, DQ, DQ, 384, 128)
                if i == NB - 1 and r == ORDER[-1]:
                    send(i, 0, DQ, 384, 128)
        for n, k in list(zip(stages[::2], stages[1::2])) + [(49, NC)]:
            for r in ORDER[:n]:
                passes.extend(P(f, r, j, done[r], k) for j in range(done[r], k))
                done[r] = k

    def run_passes(n):
        for _ in range(n):
            passes.popleft()()

    steps = dict(pin=pin, bar=barrier, mod=mod_rows, col=mod_cols, gate=gate, pq=prep_wqkv, pwo=prep_wo,
                 st1=ln1_stats, ap1=ln1_apply, ln1=lambda i: ln1_stats(i) + ln1_apply(i), qkv=qkv, qk=scores,
                 pv=mixing, proj=out_proj, ln2=ln2, pw1=prep_w1, pw2=prep_w2, up=mlp_up, down=mlp_down,
                 go=run_passes)
    named, streamed = [], {}
    for line in LINES:
        words = line.split()
        if ">" in words:
            for q in named:
                finish(q)
            for n in words[:words.index(">")]:
                while streamed.get(n) is False:
                    streamed[None].popleft()[1][2]()
                copy(n).wait()
            for n in words[words.index(">") + 1:]:
                copy(n).start()
        elif words[0] == "stream":
            dst = dict(x=(512, x_s), wo=(640, wo_s), wm=(384, wm_s), w1=(512, w1_s), w2=(512, w2_s))

            def start(n):
                copy(n).start(); streamed[n] = True
            streamed.update({n: False for n in words[1:]})
            streamed[None] = spawn([dst[n[:-1]] + (P(start, n),) for n in words[1:]],
                                   DR * sum(dst[n[:-1]][0] for n in words[1:]))
        else:
            when = [int(x) for x in words.pop(0)[1:].split("@")] if words[0][0] == "~" else None
            pieces = []
            for word in words:
                if word[0] == "!":
                    for q in {"!": named, "!1": named[-2:-1], "!!": jobs}[word]:
                        finish(q)
                    continue
                name, *args = word.split(".")
                lo, *hi = [int(x) for x in args[-1].split("-")] if args else [None]
                for last in range(lo, hi[0] + 1) if hi else [lo]:
                    new = steps[name](*[int(x) for x in args[:-1]] + [last] * bool(args)) or []
                    pieces += new
                    for p in new if when is None else ():
                        p[2]()
            if when:
                named.append(spawn(pieces, *when))
    assert not passes and not any(jobs)
    for c in sent:
        c.wait()


@jax.jit
def pallas_adaLN_cond__sliding_local_dilated__dense_activation_gelu__prompt_kernel(
        A_x, A_wqkv, A_wo, B_x, B_w1, B_b1, B_w2, B_b2, c, w_mod):
    V = pltpu.VMEM
    blocks = [V((E, TM), f32)] * NB
    out = pl.pallas_call(
        kernel,
        out_shape=jax.ShapeDtypeStruct((D, S), bf16),
        in_specs=[pl.BlockSpec(memory_space=pl.ANY)] * 9,
        out_specs=pl.BlockSpec(memory_space=pl.ANY),
        scratch_shapes=[
            V((1, D), bf16), V((F,), bf16), V((D,), bf16), V((E, S), bf16), V((E, 3 * D), bf16), V((E, D), bf16),
            V((E, F), bf16), V((E, F), bf16), V((E, 6 * D), bf16), V((D, S), bf16),
            V((5, 3 * D // 2 + 16, 128), u32), V((5, E + 16, 128), f32), V((5, E, 128), f32),
            V((96, 384), f32), V((6 * D + 16, 128), f32),
            blocks, blocks, blocks, V((2, D, 128), f32), V((2, D, 128), f32), V((2, 4, 4, 8, 128), f32),
            V((NT, 4, W, 8, 128), f32), blocks[:2], V((53, 144, 128), bf16), V((53, 64, 128), u32),
            V((NC, 49, 128, 128), bf16), V((NC, 4, 128, 128), bf16), V((NC, 49, DQ, 128), bf16),
            [V((49, 128, 128), bf16)] * NC, V((49, DQ, 128), f32), [[V((4, 144, 128), f32)] * 4] * NC,
            V((2 * NS, DQ, 128), f32), [V((16, D // 2, 128), bf16)] * 4, [V((2, 16, 128, 128), bf16)] * 3,
            V((2, 16, 128, 128), bf16),
            pltpu.SemaphoreType.DMA((len(WAITS),)), pltpu.SemaphoreType.DMA, pltpu.SemaphoreType.REGULAR,
            pltpu.SemaphoreType.REGULAR,
        ],
        compiler_params=pltpu.CompilerParams(vmem_limit_bytes=127 * 2**20),
    )(c, B_b1, B_b2, A_x.reshape(S, D).T, A_wqkv, A_wo, B_w1, B_w2.T, w_mod)
    return out.T.reshape(1, S, D)
```
